```python
import os as _os
_os.environ.setdefault("JAX_PLATFORMS", "cpu")
import jax
import jax.numpy as jnp

def _softmax(x, axis=-1):
    return jax.nn.softmax(x, axis=axis)
def _gelu(x):
    return jax.nn.gelu(x, approximate=True)
def _silu(x):
    return jax.nn.silu(x)
def _sigmoid(x):
    return jax.nn.sigmoid(x)
def _layernorm(x, axis=-1, eps=1e-5):
    m = jnp.mean(x, axis=axis, keepdims=True)
    v = jnp.var(x, axis=axis, keepdims=True)
    return (x - m) / jnp.sqrt(v + eps)
def _scatter_add(tgt, idx, src, axis=0):
    return tgt.at[idx].add(src)
def _segment_sum(src, seg, n):
    return jax.ops.segment_sum(src, seg, n)
class _Rng:
    def __init__(self, key):
        self._k = key
    def _next(self):
        self._k, sub = jax.random.split(self._k)
        return sub
    def normal(self, shape):
        return jax.random.normal(self._next(), shape, dtype=jnp.bfloat16)
    def randint(self, lo, hi, shape):
        return jax.random.randint(self._next(), shape, lo, hi, dtype=jnp.int32)
    def uniform(self, shape, lo=0.0, hi=1.0):
        return jax.random.uniform(self._next(), shape, jnp.bfloat16, lo, hi)
    def permutation(self, n):
        return jax.random.permutation(self._next(), n)


kernel_name = 'standalone__mha_softmax__near_ridge'

def setup_inputs():
    _rng = _Rng(jax.random.key(int.from_bytes(__import__("os").urandom(4), "little")))
    _w = (lambda a: (lambda t: t.astype(jnp.bfloat16) if jnp.issubdtype(t.dtype, jnp.floating) else t)(jnp.asarray(a)))
    B, H, Sq, Sk, D = 8, 32, 304, 2048, 128
    return {
        "q": _w((lambda *s: _rng.normal(s) * 0.4)(B, H, Sq, D)),
        "k": _w((lambda *s: _rng.normal(s) * 0.4)(B, H, Sk, D)),
        "v": _w((lambda *s: _rng.normal(s) * 0.05)(B, H, Sk, D)),
    }

def reference(q, k, v):
    scale = q.shape[-1] ** -0.5
    scores = jnp.einsum("bhqd,bhkd->bhqk", q, k) * scale
    p = _softmax(scores, axis=-1)
    return jnp.einsum("bhqk,bhkd->bhqd", p, v)
```

```python
import jax
import jax.numpy as jnp
import jax.experimental.pallas as pl
import jax.experimental.pallas.tpu as pltpu

_LOG2E = 1.4426950408889634
_G = 8
_DIST = 3
_FIN_TILE = 4


def _kernel(q_hbm, k_hbm, v_hbm, o_hbm, qb, kb, vb, ob, ab, lb, one, sems, osem):
    N, Sq, D = q_hbm.shape
    Sk = k_hbm.shape[1]
    G, d = _G, _DIST
    NT = Sk // 128
    n_it = N // G
    c = (D ** -0.5) * _LOG2E

    def q_cp(h, s):
        return pltpu.make_async_copy(q_hbm.at[h], qb.at[s], sems.at[0, s])

    def k_cp(h, s):
        return pltpu.make_async_copy(k_hbm.at[h], kb.at[s], sems.at[1, s])

    def v_cp(h, s):
        return pltpu.make_async_copy(v_hbm.at[h], vb.at[s], sems.at[2, s])

    def o_cp(j):
        return pltpu.make_async_copy(ob.at[j % 2], o_hbm.at[pl.ds(j * G - 1, G)], osem.at[j % 2])

    def o_cp_first():
        return pltpu.make_async_copy(ob.at[0, pl.ds(1, G - 1)], o_hbm.at[pl.ds(0, G - 1)], osem.at[0])

    def o_cp_last():
        return pltpu.make_async_copy(ob.at[n_it % 2, 0], o_hbm.at[N - 1], osem.at[n_it % 2])

    def ld(ref, s):
        return pltpu.bitcast(ref.bitcast(jnp.uint32)[s], jnp.bfloat16)

    def recip(l):
        r = pltpu.reciprocal(l, approx=True)
        return r * (2.0 - l * r)

    def scores(s):
        sc = jax.lax.dot_general(ld(qb, s), ld(kb, s), (((1,), (1,)), ((), ())),
                                 preferred_element_type=jnp.float32)
        m = jnp.broadcast_to(jnp.max(sc, axis=1, keepdims=True), (Sq, D))
        return sc, m

    def weighted(sc, m, s, flag, prev):
        p = jnp.exp2((sc - jnp.concatenate([m] * NT, axis=1)) * c)
        ts = [p[:, t * 128:(t + 1) * 128] for t in range(NT)]
        lpart = ts[0]
        for t in range(1, NT):
            lpart = lpart + ts[t]
        ts[_FIN_TILE] = jnp.where(flag, ts[_FIN_TILE], prev)
        p = jnp.concatenate(ts, axis=1).astype(jnp.bfloat16)
        acc = jnp.dot(p, ld(vb, s), preferred_element_type=jnp.float32)
        return acc, lpart

    def normalise(acc, lpart):
        return acc * recip(jnp.sum(lpart, axis=1, keepdims=True))

    one[0] = 1
    ab[...] = jnp.zeros(ab.shape, ab.dtype)
    lb[...] = jnp.ones(lb.shape, lb.dtype)
    for h in range(d):
        q_cp(h, h).start()
        k_cp(h, h).start()
        v_cp(h, h).start()

    def body(i, carry):
        @pl.when(i == 2)
        def _():
            o_cp_first().wait()

        @pl.when(i > 2)
        def _():
            o_cp(i - 2).wait()

        flag = one[0] > 0
        prev = normalise(ab[...], lb[...])
        ob[i % 2, 0] = prev.astype(ob.dtype)
        for g in range(G):
            h = i * G + g
            hp = jnp.minimum(h + d, N - 1)
            s_pre = (g + d) % G
            q_cp(hp, s_pre).start()
            k_cp(hp, s_pre).start()
            v_cp(hp, s_pre).start()
            q_cp(h, g).wait()
            k_cp(h, g).wait()
            sc, m = scores(g)
            v_cp(h, g).wait()
            acc, lpart = weighted(sc, m, g, flag, prev)
            if g == G - 1:
                ab[...] = acc
                lb[...] = lpart
            else:
                prev = normalise(acc, lpart)
                ob[i % 2, g + 1] = prev.astype(ob.dtype)

        @pl.when(i == 0)
        def _():
            o_cp_first().start()

        @pl.when(i > 0)
        def _():
            o_cp(i).start()

        return carry

    jax.lax.fori_loop(0, n_it, body, 0)
    o_cp(n_it - 2).wait()
    ob[n_it % 2, 0] = normalise(ab[...], lb[...]).astype(ob.dtype)
    o_cp_last().start()
    for s in range(d):
        q_cp(N - 1, s).wait()
        k_cp(N - 1, s).wait()
        v_cp(N - 1, s).wait()
    o_cp(n_it - 1).wait()
    o_cp_last().wait()


@jax.jit
def pallas_standalone__mha_softmax__near_ridge_kernel(
    q: jax.Array,
    k: jax.Array,
    v: jax.Array,
):
    B, H, Sq, D = q.shape
    Sk = k.shape[2]
    N = B * H
    G = _G
    assert N % G == 0 and N // G >= 3 and Sk % 128 == 0
    out = pl.pallas_call(
        _kernel,
        in_specs=[pl.BlockSpec(memory_space=pl.ANY)] * 3,
        out_specs=pl.BlockSpec(memory_space=pl.ANY),
        out_shape=jax.ShapeDtypeStruct((N, Sq, D), q.dtype),
        scratch_shapes=[
            pltpu.VMEM((G, Sq, D), q.dtype),
            pltpu.VMEM((G, Sk, D), k.dtype),
            pltpu.VMEM((G, Sk, D), v.dtype),
            pltpu.VMEM((2, G, Sq, D), q.dtype),
            pltpu.VMEM((Sq, D), jnp.float32),
            pltpu.VMEM((Sq, D), jnp.float32),
            pltpu.SMEM((1,), jnp.int32),
            pltpu.SemaphoreType.DMA((3, G)),
            pltpu.SemaphoreType.DMA((2,)),
        ],
        compiler_params=pltpu.CompilerParams(
            vmem_limit_bytes=100 * 1024 * 1024,
            flags={"XLA_TPU_RESCHEDULE_DMA_DONES": True},
        ),
    )(q.reshape(N, Sq, D), k.reshape(N, Sk, D), v.reshape(N, Sk, D))
    return out.reshape(B, H, Sq, D)
```

```python
import jax
import jax.numpy as jnp
import jax.experimental.pallas as pl
import jax.experimental.pallas.tpu as pltpu

_LOG2E = 1.4426950408889634
_G = 16
_DIST = 3
_LANES = 128
_KBLK = 4


def _kernel(q_hbm, k_hbm, v_hbm, o_hbm, qb, kb, vb, ob, ab, lb, one, sems, osem):
    N, Sq, D = q_hbm.shape
    Sk = k_hbm.shape[1]
    G, d = _G, _DIST
    NT = Sk // _LANES
    CK = Sk // _KBLK
    n_it = N // G
    c = (D ** -0.5) * _LOG2E

    def q_cp(h, s):
        return pltpu.make_async_copy(q_hbm.at[h], qb.at[s], sems.at[0, s])

    def k_cp(h, s):
        return pltpu.make_async_copy(k_hbm.at[h], kb.at[s], sems.at[1, s])

    def v_cp(h, s):
        return pltpu.make_async_copy(v_hbm.at[h], vb.at[s], sems.at[2, s])

    def o_cp(j):
        return pltpu.make_async_copy(ob.at[j % 2], o_hbm.at[pl.ds(j * G - 1, G)], osem.at[j % 2])

    def o_cp_first():
        return pltpu.make_async_copy(ob.at[0, pl.ds(1, G - 1)], o_hbm.at[pl.ds(0, G - 1)], osem.at[0])

    def o_cp_last():
        return pltpu.make_async_copy(ob.at[n_it % 2, 0], o_hbm.at[N - 1], osem.at[n_it % 2])

    def ld(ref, s):
        return pltpu.bitcast(ref.bitcast(jnp.uint32)[s], jnp.bfloat16)

    def nt_dot(a, b):
        return jax.lax.dot_general(a, b, (((1,), (1,)), ((), ())), preferred_element_type=jnp.float32)

    def normalise(acc, lpart):
        l = jnp.sum(lpart, axis=1, keepdims=True)
        r = pltpu.reciprocal(l, approx=True)
        r = r * (2.0 - l * r)
        return (acc * r).astype(ob.dtype)


    def scores(s, flag, pending, store_prev):
        q = ld(qb, s)
        k = ld(kb, s)
        head = [nt_dot(q, k[j * CK:(j + 1) * CK]) for j in range(_KBLK - 1)]
        acc, lpart = pending
        prev = normalise(acc, jnp.where(flag, lpart, head[0][:, :_LANES]))
        store_prev(prev)
        q_tied = pltpu.bitcast(
            jnp.where(flag, pltpu.bitcast(q, jnp.uint32), pltpu.bitcast(prev, jnp.uint32)), jnp.bfloat16)
        sc = jnp.concatenate(head + [nt_dot(q_tied, k[(_KBLK - 1) * CK:])], axis=1)
        m = jnp.broadcast_to(jnp.max(sc, axis=1, keepdims=True), (Sq, _LANES))
        return sc, m

    def weighted(sc, m, s, flag):
        p = jnp.exp2((sc - jnp.concatenate([m] * NT, axis=1)) * c)
        ts = [p[:, t * _LANES:(t + 1) * _LANES] for t in range(NT)]
        lpart = None
        for t in range(0, NT, 4):
            x = (ts[t] + ts[t + 1]) + (ts[t + 2] + ts[t + 3])
            lpart = x if lpart is None else lpart + x
            ts[t + 3] = jnp.where(flag, ts[t + 3], lpart)
        p = jnp.concatenate(ts, axis=1).astype(jnp.bfloat16)
        acc = jnp.dot(p, ld(vb, s), preferred_element_type=jnp.float32)
        return acc, lpart

    one[0] = 1
    ab[...] = jnp.zeros(ab.shape, ab.dtype)
    lb[...] = jnp.ones(lb.shape, lb.dtype)
    q_cp(0, 0).start()
    k_cp(0, 0).start()
    v_cp(0, 0).start()
    q_cp(0, 0).wait()
    k_cp(0, 0).wait()
    for h in range(1, d):
        q_cp(h, h).start()
        k_cp(h, h).start()
        v_cp(h, h).start()

    def body(i, carry):
        @pl.when(i == 2)
        def _():
            o_cp_first().wait()

        @pl.when(i > 2)
        def _():
            o_cp(i - 2).wait()

        flag = one[0] > 0
        pending = (ab[...], lb[...])
        for g in range(G):
            h = i * G + g
            hp = jnp.minimum(h + d, N - 1)
            s_pre = (g + d) % G
            q_cp(hp, s_pre).start()
            k_cp(hp, s_pre).start()
            v_cp(hp, s_pre).start()
            if g == 0:
                @pl.when(i > 0)
                def _():
                    q_cp(h, g).wait()
                    k_cp(h, g).wait()
            else:
                q_cp(h, g).wait()
                k_cp(h, g).wait()

            def store_prev(x, g=g):
                ob[i % 2, g] = x

            sc, m = scores(g, flag, pending, store_prev)
            v_cp(h, g).wait()
            pending = weighted(sc, m, g, flag)
        ab[...] = pending[0]
        lb[...] = pending[1]

        @pl.when(i == 0)
        def _():
            o_cp_first().start()

        @pl.when(i > 0)
        def _():
            o_cp(i).start()

        return carry

    jax.lax.fori_loop(0, n_it, body, 0)

    o_cp(n_it - 2).wait()
    ob[n_it % 2, 0] = normalise(ab[...], lb[...])
    o_cp_last().start()
    for s in range(d):
        q_cp(N - 1, s).wait()
        k_cp(N - 1, s).wait()
        v_cp(N - 1, s).wait()
    o_cp(n_it - 1).wait()
    o_cp_last().wait()


@jax.jit
def pallas_standalone__mha_softmax__near_ridge_kernel(
    q: jax.Array,
    k: jax.Array,
    v: jax.Array,
):
    B, H, Sq, D = q.shape
    Sk = k.shape[2]
    N = B * H
    G = _G
    assert N % G == 0 and N // G >= 3 and D == _LANES and Sq % 16 == 0 and Sk % (4 * _KBLK * _LANES // 4) == 0
    out = pl.pallas_call(
        _kernel,
        in_specs=[pl.BlockSpec(memory_space=pl.ANY)] * 3,
        out_specs=pl.BlockSpec(memory_space=pl.ANY),
        out_shape=jax.ShapeDtypeStruct((N, Sq, D), q.dtype),
        scratch_shapes=[
            pltpu.VMEM((G, Sq, D), q.dtype),
            pltpu.VMEM((G, Sk, D), k.dtype),
            pltpu.VMEM((G, Sk, D), v.dtype),
            pltpu.VMEM((2, G, Sq, D), q.dtype),
            pltpu.VMEM((Sq, D), jnp.float32),
            pltpu.VMEM((Sq, _LANES), jnp.float32),
            pltpu.SMEM((1,), jnp.int32),
            pltpu.SemaphoreType.DMA((3, G)),
            pltpu.SemaphoreType.DMA((2,)),
        ],
        compiler_params=pltpu.CompilerParams(
            vmem_limit_bytes=100 * 1024 * 1024,
            disable_bounds_checks=True,
            flags={"XLA_TPU_RESCHEDULE_DMA_DONES": True},
        ),
    )(q.reshape(N, Sq, D), k.reshape(N, Sk, D), v.reshape(N, Sk, D))
    return out.reshape(B, H, Sq, D)
```

```python
import jax
import jax.numpy as jnp
import jax.experimental.pallas as pl
import jax.experimental.pallas.tpu as pltpu

_LOG2E = 1.4426950408889634
_LANES = 128
_G = 16
_R = 4
_DIST = 3
_W = 8


def _kernel(q_hbm, k_hbm, v_hbm, o_hbm, qb, kb, vb, ob, ab, lb, one, sems, osem):
    N, Sq, D = q_hbm.shape
    Sk = k_hbm.shape[1]
    G, R, d, W = _G, _R, _DIST, _W
    NT = Sk // _LANES
    KSPLIT = 3 * Sk // 4
    n_it = N // G
    c = (D ** -0.5) * _LOG2E

    def q_cp(h, s):
        return pltpu.make_async_copy(q_hbm.at[h], qb.at[s], sems.at[0, s])

    def k_cp(h, s):
        return pltpu.make_async_copy(k_hbm.at[h], kb.at[s], sems.at[1, s])

    def v_cp(h, s):
        return pltpu.make_async_copy(v_hbm.at[h], vb.at[s], sems.at[2, s])

    def start_inputs(h, s):
        q_cp(h, s).start()
        k_cp(h, s).start()
        v_cp(h, s).start()

    def o_cp(i, w):
        return pltpu.make_async_copy(ob.at[w], o_hbm.at[pl.ds(i * G + w * W - 1, W)], osem.at[w])

    def o_cp_first():
        return pltpu.make_async_copy(ob.at[0, pl.ds(1, W - 1)], o_hbm.at[pl.ds(0, W - 1)], osem.at[0])

    def o_cp_last():
        return pltpu.make_async_copy(ob.at[0, 0], o_hbm.at[N - 1], osem.at[0])

    def nt_dot(a, b):
        return jax.lax.dot_general(a, b, (((1,), (1,)), ((), ())), preferred_element_type=jnp.float32)

    def normalise(acc, lpart):
        l = jnp.sum(lpart, axis=1, keepdims=True)
        return (acc * (1.0 / l)).astype(ob.dtype)

    def scores(s, flag, pending):
        q = qb[s]
        k = kb[s]
        first = nt_dot(q, k[:KSPLIT])
        acc, lpart = pending
        prev = normalise(acc, jnp.where(flag, lpart, first[:, _LANES:2 * _LANES]))
        q_tied = pltpu.bitcast(
            jnp.where(flag, pltpu.bitcast(q, jnp.uint32), pltpu.bitcast(prev, jnp.uint32)), q.dtype)
        sc = jnp.concatenate([first, nt_dot(q_tied, k[KSPLIT:])], axis=1)
        m = jnp.broadcast_to(jnp.max(sc, axis=1, keepdims=True), (Sq, _LANES))
        return sc, m, prev

    def weighted(sc, m, s):
        p = jnp.exp2((jnp.concatenate([m] * NT, axis=1) - sc) * (-c))
        tiles = [p[:, t * _LANES:(t + 1) * _LANES] for t in range(NT)]
        lpart = tiles[0]
        for t in range(1, NT):
            lpart = lpart + tiles[t]
        pb = jnp.concatenate([t.astype(vb.dtype) for t in tiles], axis=1)
        acc = jnp.dot(pb, vb[s], preferred_element_type=jnp.float32)
        return acc, lpart

    one[0] = 1
    ab[...] = jnp.zeros(ab.shape, ab.dtype)
    lb[...] = jnp.ones(lb.shape, lb.dtype)
    start_inputs(0, 0)
    q_cp(0, 0).wait()
    k_cp(0, 0).wait()
    for h in range(1, d):
        start_inputs(h, h)

    def body(i, carry):
        flag = one[0] > 0
        pending = (ab[...], lb[...])
        for g in range(G):
            h = i * G + g
            s = g % R
            w = g // W
            if g % W == 0:
                if w == 0:
                    pl.when(i == 1)(lambda: o_cp_first().wait())
                    pl.when(i > 1)(lambda: o_cp(i - 1, 0).wait())
                else:
                    pl.when(i > 0)(lambda w=w: o_cp(i - 1, w).wait())
            if g + d < G:
                start_inputs(h + d, (g + d) % R)
            else:
                pl.when(i < n_it - 1)(lambda g=g, h=h: start_inputs(h + d, (g + d) % R))
            if g == 0:
                @pl.when(i > 0)
                def _():
                    q_cp(h, s).wait()
                    k_cp(h, s).wait()
            else:
                q_cp(h, s).wait()
                k_cp(h, s).wait()
            sc, m, prev = scores(s, flag, pending)
            ob[w, g % W] = prev
            v_cp(h, s).wait()
            pending = weighted(sc, m, s)
            if g % W == W - 1:
                if w == 0:
                    pl.when(i == 0)(lambda: o_cp_first().start())
                    pl.when(i > 0)(lambda: o_cp(i, 0).start())
                else:
                    o_cp(i, w).start()
        ab[...] = pending[0]
        lb[...] = pending[1]
        return carry

    jax.lax.fori_loop(0, n_it, body, 0)

    o_cp(n_it - 1, 0).wait()
    ob[0, 0] = normalise(ab[...], lb[...])
    o_cp_last().start()
    for w in range(1, G // W):
        o_cp(n_it - 1, w).wait()
    o_cp_last().wait()


@jax.jit
def pallas_standalone__mha_softmax__near_ridge_kernel(
    q: jax.Array,
    k: jax.Array,
    v: jax.Array,
):
    B, H, Sq, D = q.shape
    Sk = k.shape[2]
    N = B * H
    assert N % _G == 0 and N // _G >= 2
    assert D == _LANES and Sq % 16 == 0 and Sk % (4 * _LANES) == 0 and Sk >= 8 * _LANES
    out = pl.pallas_call(
        _kernel,
        in_specs=[pl.BlockSpec(memory_space=pl.ANY)] * 3,
        out_specs=pl.BlockSpec(memory_space=pl.ANY),
        out_shape=jax.ShapeDtypeStruct((N, Sq, D), q.dtype),
        scratch_shapes=[
            pltpu.VMEM((_R, Sq, D), q.dtype),
            pltpu.VMEM((_R, Sk, D), k.dtype),
            pltpu.VMEM((_R, Sk, D), v.dtype),
            pltpu.VMEM((_G // _W, _W, Sq, D), q.dtype),
            pltpu.VMEM((Sq, D), jnp.float32),
            pltpu.VMEM((Sq, _LANES), jnp.float32),
            pltpu.SMEM((1,), jnp.int32),
            pltpu.SemaphoreType.DMA((3, _R)),
            pltpu.SemaphoreType.DMA((_G // _W,)),
        ],
        compiler_params=pltpu.CompilerParams(
            vmem_limit_bytes=100 * 1024 * 1024,
            flags={"XLA_TPU_RESCHEDULE_DMA_DONES": True},
        ),
    )(q.reshape(N, Sq, D), k.reshape(N, Sk, D), v.reshape(N, Sk, D))
    return out.reshape(B, H, Sq, D)
```
